```python
import jax
import jax.numpy as jnp

def _softmax(x, axis=-1):
    return jax.nn.softmax(x, axis=axis)

def _gelu(x):
    return jax.nn.gelu(x, approximate=True)

def _silu(x):
    return jax.nn.silu(x)

def _sigmoid(x):
    return jax.nn.sigmoid(x)

def _layernorm(x, axis=-1, eps=1e-05):
    m = jnp.mean(x, axis=axis, keepdims=True)
    v = jnp.var(x, axis=axis, keepdims=True)
    return (x - m) / jnp.sqrt(v + eps)

def _scatter_add(tgt, idx, src, axis=0):
    return tgt.at[idx].add(src)

def _segment_sum(src, seg, n):
    return jax.ops.segment_sum(src, seg, n)

class _Rng:

    def __init__(self, key):
        self._k = key

    def _next(self):
        self._k, sub = jax.random.split(self._k)
        return sub

    def normal(self, shape):
        return jax.random.normal(self._next(), shape, dtype=jnp.bfloat16)

    def randint(self, lo, hi, shape):
        return jax.random.randint(self._next(), shape, lo, hi, dtype=jnp.int32)

    def uniform(self, shape, lo=0.0, hi=1.0):
        return jax.random.uniform(self._next(), shape, jnp.bfloat16, lo, hi)

    def permutation(self, n):
        return jax.random.permutation(self._next(), n)
kernel_name = 'adaLN_cond__sliding_block_cached__mixer_channel_mlp__decode'

def setup_inputs():
    _rng = _Rng(jax.random.key(int.from_bytes(__import__("os").urandom(4), "little")))
    _w = lambda a: (lambda t: t.astype(jnp.bfloat16) if jnp.issubdtype(t.dtype, jnp.floating) else t)(jnp.asarray(a))

    def _A_setup():
        B, Sq, D = (8, 1, 640)
        Hq, Hkv, Sk, Dh = (32, 32, 4096, 192)
        assert Hq % Hkv == 0, (Hq, Hkv)
        return {'x': _w((lambda *s: _rng.normal(s) * 0.05)(B, Sq, D)), 'k_cache': _w((lambda *s: _rng.normal(s) * 0.05)(B, Hkv, Sk, Dh)), 'v_cache': _w((lambda *s: _rng.normal(s) * 0.05)(B, Hkv, Sk, Dh)), 'wq': _w((lambda *s: _rng.normal(s) * 0.05)(D, Hq * Dh) * D ** (-0.5)), 'wo': _w((lambda *s: _rng.normal(s) * 0.05)(Hq * Dh, D) * (Hq * Dh) ** (-0.5))}
    _A_in = _A_setup()

    def _B_setup():
        B, S, D, F = (8, 1, 640, 1536)
        return {'x': _w((lambda *s: _rng.normal(s) * 0.05)(B, S, D)), 'w1': _w((lambda *s: _rng.normal(s) * 0.05)(D, F) * D ** (-0.5)), 'b1': _w((lambda *s: _rng.normal(s) * 0.05)(F)), 'w2': _w((lambda *s: _rng.normal(s) * 0.05)(F, D) * F ** (-0.5)), 'b2': _w((lambda *s: _rng.normal(s) * 0.05)(D))}
    _B_in = _B_setup()
    return {'A_x': _A_in['x'], 'A_k_cache': _A_in['k_cache'], 'A_v_cache': _A_in['v_cache'], 'A_wq': _A_in['wq'], 'A_wo': _A_in['wo'], 'B_x': _B_in['x'], 'B_w1': _B_in['w1'], 'B_b1': _B_in['b1'], 'B_w2': _B_in['w2'], 'B_b2': _B_in['b2'], 'c': _w((lambda *s: _rng.normal(s) * 0.05)(8, 640)), 'w_mod': _w((lambda *s: _rng.normal(s) * 0.05)(640, 6 * 640) * 640 ** (-0.5))}

def reference(A_x, A_k_cache, A_v_cache, A_wq, A_wo, B_x, B_w1, B_b1, B_w2, B_b2, c, w_mod):

    def _A_ref(x, k_cache, v_cache, wq, wo):
        B, Sq, D = x.shape
        Hq, Dh = (32, 192)
        Hkv, Sk = (k_cache.shape[1], k_cache.shape[2])
        W = min(4096, max(256, Sk // 4))
        rep = Hq // Hkv
        q = (lambda x, *d: x.transpose(*d))((x @ wq).reshape(B, Sq, Hq, Dh), 0, 2, 1, 3)
        k = jnp.repeat(k_cache[:, :, Sk - W:, :], rep, axis=1)
        v = jnp.repeat(v_cache[:, :, Sk - W:, :], rep, axis=1)
        scores = jnp.einsum('bhqd,bhkd->bhqk', q, k) * Dh ** (-0.5)
        p = _softmax(scores, axis=-1)
        o = jnp.einsum('bhqk,bhkd->bhqd', p, v)
        return (lambda x, *d: x.transpose(*d))(o, 0, 2, 1, 3).reshape(B, Sq, Hq * Dh) @ wo

    def _B_ref(x, w1, b1, w2, b2):
        y = _layernorm(x, axis=-1)
        h = _gelu(jnp.einsum('bsd,df->bsf', y, w1) + b1)
        return jnp.einsum('bsf,fd->bsd', h, w2) + b2
    x = A_x
    mod = (_silu(c) @ w_mod).reshape(c.shape[0], 6, 1, -1)
    sa, ca, ga, sb, cb, gb = (mod[:, 0].copy(), mod[:, 1].copy(), mod[:, 2].copy(), mod[:, 3].copy(), mod[:, 4].copy(), mod[:, 5].copy())
    h = _layernorm(x, axis=-1) * (1 + ca) + sa
    x = x + ga * _A_ref(h, A_k_cache, A_v_cache, A_wq, A_wo)
    h = _layernorm(x, axis=-1) * (1 + cb) + sb
    x = x + gb * _B_ref(h, B_w1, B_b1, B_w2, B_b2)
    return x
```

```python
import functools
import jax
import jax.numpy as jnp
from jax.experimental import pallas as pl
from jax.experimental.pallas import tpu as pltpu

F32 = jnp.float32
BF16 = jnp.bfloat16


def _layernorm(x, eps=1e-5):
    m = jnp.mean(x, axis=-1, keepdims=True)
    d = x - m
    v = jnp.mean(d * d, axis=-1, keepdims=True)
    return d / jnp.sqrt(v + eps)


def _dot(a, b):
    return jnp.dot(a, b, preferred_element_type=F32)


def make(NBUF=4, HG=8):
    def fn(A_x, A_k_cache, A_v_cache, A_wq, A_wo, B_x, B_w1, B_b1, B_w2, B_b2, c, w_mod):
        B, Sq, D = A_x.shape
        _, H, Sk, Dh = A_k_cache.shape
        Fh = B_w1.shape[1]
        W = min(4096, max(256, Sk // 4))
        R = HG * Dh
        NG = H // HG
        NSTEP = NG * B
        scale = Dh ** -0.5

        def kernel(x_hbm, k_hbm, v_hbm, wq_hbm, wo_hbm, w1_hbm, b1_hbm, w2_hbm, b2_hbm, c_hbm, wmod_hbm,
                   out_ref,
                   x_v, c_v, b1_v, b2_v, wmod_v, wq_v, wo_v, w1_v, w2_v, k_v, v_v, q_v,
                   sem_w, sem_q, sem_o, sem_k, sem_v):
            def kv_copy(src, dst, sem, step, slot):
                g = step // B
                b = step % B
                return pltpu.make_async_copy(
                    src.at[b, pl.ds(pl.multiple_of(g * R, R), R), pl.ds(Sk - W, W)], dst.at[slot], sem.at[slot])

            cp_c = pltpu.make_async_copy(c_hbm, c_v, sem_w.at[0])
            cp_x = pltpu.make_async_copy(x_hbm, x_v, sem_w.at[1])
            cp_moda = pltpu.make_async_copy(wmod_hbm.at[:, pl.ds(0, 2 * D)], wmod_v.at[:, pl.ds(0, 2 * D)], sem_w.at[2])
            cp_modb = pltpu.make_async_copy(wmod_hbm.at[:, pl.ds(2 * D, 4 * D)], wmod_v.at[:, pl.ds(2 * D, 4 * D)], sem_w.at[3])
            cp_b1 = pltpu.make_async_copy(b1_hbm, b1_v, sem_w.at[4])
            cp_b2 = pltpu.make_async_copy(b2_hbm, b2_v, sem_w.at[5])
            cp_w1 = pltpu.make_async_copy(w1_hbm, w1_v, sem_w.at[6])
            cp_w2 = pltpu.make_async_copy(w2_hbm, w2_v, sem_w.at[7])
            cp_wq = [pltpu.make_async_copy(wq_hbm.at[:, pl.ds(g * R, R)], wq_v.at[g], sem_q.at[g]) for g in range(NG)]
            cp_wo = [pltpu.make_async_copy(wo_hbm.at[pl.ds(g * R, R), :], wo_v.at[g], sem_o.at[g]) for g in range(NG)]

            cp_c.start()
            cp_x.start()
            cp_moda.start()
            cp_wq[0].start()
            for s in range(NBUF):
                kv_copy(k_hbm, k_v, sem_k, s, s).start()
                kv_copy(v_hbm, v_v, sem_v, s, s).start()
            for g in range(1, NG):
                cp_wq[g].start()
            for g in range(NG):
                cp_wo[g].start()
            cp_modb.start()
            cp_b1.start()
            cp_b2.start()
            cp_w1.start()
            cp_w2.start()

            cp_c.wait()
            cc = c_v[...].astype(F32)
            sc = (cc * jax.nn.sigmoid(cc)).astype(BF16)
            cp_x.wait()
            x = x_v[...].astype(F32)
            xn = _layernorm(x)
            cp_moda.wait()
            moda = _dot(sc, wmod_v[:, 0:2 * D])
            h = (xn * (1.0 + moda[:, D:2 * D]) + moda[:, 0:D]).astype(BF16)

            row = jax.lax.broadcasted_iota(jnp.int32, (B, R), 0)
            col = jax.lax.broadcasted_iota(jnp.int32, (B, R), 1)

            attn = jnp.zeros((B, D), F32)
            for g in range(NG):
                cp_wq[g].wait()
                q_v[...] = _dot(h, wq_v[g])

                def body(b, o_all):
                    step = g * B + b
                    slot = step % NBUF
                    diag = (col >= row * Dh) & (col < (row + 1) * Dh)
                    qb = jnp.broadcast_to(q_v[pl.ds(b, 1), :], (HG, R))
                    qd = jnp.where(diag, qb, 0.0).astype(BF16)
                    kv_copy(k_hbm, k_v, sem_k, step, slot).wait()
                    s = _dot(qd, k_v[slot]) * scale

                    @pl.when(step + NBUF < NSTEP)
                    def _():
                        kv_copy(k_hbm, k_v, sem_k, step + NBUF, slot).start()

                    m = jnp.max(s, axis=-1, keepdims=True)
                    e = jnp.exp(s - m)
                    l = jnp.sum(e, axis=-1, keepdims=True)
                    kv_copy(v_hbm, v_v, sem_v, step, slot).wait()
                    o = jax.lax.dot_general(e.astype(BF16), v_v[slot], (((1,), (1,)), ((), ())),
                                            preferred_element_type=F32)

                    @pl.when(step + NBUF < NSTEP)
                    def _():
                        kv_copy(v_hbm, v_v, sem_v, step + NBUF, slot).start()

                    o = jnp.where(diag, o / l, 0.0)
                    orow = jnp.sum(o, axis=0, keepdims=True)
                    return jnp.where(row == b, orow, o_all)

                o_all = jax.lax.fori_loop(0, B, body, jnp.zeros((B, R), F32))
                cp_wo[g].wait()
                attn = attn + _dot(o_all.astype(BF16), wo_v[g])

            cp_modb.wait()
            modb = _dot(sc, wmod_v[:, 2 * D:6 * D])
            ga, sb, cb, gb = (modb[:, i * D:(i + 1) * D] for i in range(4))
            x1 = x + ga * attn
            h2 = _layernorm(x1) * (1.0 + cb) + sb
            y = _layernorm(h2).astype(BF16)
            cp_b1.wait()
            cp_w1.wait()
            u = _dot(y, w1_v[...]) + b1_v[...].astype(F32)[None, :]
            u = jax.nn.gelu(u, approximate=True).astype(BF16)
            cp_b2.wait()
            cp_w2.wait()
            mlp = _dot(u, w2_v[...]) + b2_v[...].astype(F32)[None, :]
            out_ref[...] = (x1 + gb * mlp).astype(out_ref.dtype)

        kt = jnp.swapaxes(A_k_cache, 2, 3).reshape(B, H * Dh, Sk)
        vt = jnp.swapaxes(A_v_cache, 2, 3).reshape(B, H * Dh, Sk)
        out = pl.pallas_call(
            kernel,
            out_shape=jax.ShapeDtypeStruct((B, D), A_x.dtype),
            in_specs=[pl.BlockSpec(memory_space=pl.ANY)] * 11,
            out_specs=pl.BlockSpec(memory_space=pltpu.VMEM),
            scratch_shapes=[
                pltpu.VMEM((B, D), BF16), pltpu.VMEM((B, D), BF16),
                pltpu.VMEM((Fh,), BF16), pltpu.VMEM((D,), BF16),
                pltpu.VMEM((D, 6 * D), BF16), pltpu.VMEM((NG, D, R), BF16), pltpu.VMEM((NG, R, D), BF16),
                pltpu.VMEM((D, Fh), BF16), pltpu.VMEM((Fh, D), BF16),
                pltpu.VMEM((NBUF, R, W), BF16), pltpu.VMEM((NBUF, R, W), BF16),
                pltpu.VMEM((B, R), F32),
                pltpu.SemaphoreType.DMA((8,)), pltpu.SemaphoreType.DMA((NG,)), pltpu.SemaphoreType.DMA((NG,)),
                pltpu.SemaphoreType.DMA((NBUF,)), pltpu.SemaphoreType.DMA((NBUF,)),
            ],
            compiler_params=pltpu.CompilerParams(vmem_limit_bytes=110 * 1024 * 1024),
        )(A_x.reshape(B, D), kt, vt, A_wq, A_wo, B_w1, B_b1, B_w2, B_b2, c, w_mod)
        return out.reshape(B, Sq, D)
    return fn


_impl = make()


@jax.jit
def pallas_adaLN_cond__sliding_block_cached__mixer_channel_mlp__decode_kernel(
    A_x, A_k_cache, A_v_cache, A_wq, A_wo, B_x, B_w1, B_b1, B_w2, B_b2, c, w_mod
):
    return _impl(A_x, A_k_cache, A_v_cache, A_wq, A_wo, B_x, B_w1, B_b1, B_w2, B_b2, c, w_mod)
```

```python
import functools
import jax
import jax.numpy as jnp
from jax.experimental import pallas as pl
from jax.experimental.pallas import tpu as pltpu

F32 = jnp.float32
BF16 = jnp.bfloat16


def _layernorm(x, eps=1e-5):
    m = jnp.mean(x, axis=-1, keepdims=True)
    d = x - m
    v = jnp.mean(d * d, axis=-1, keepdims=True)
    return d / jnp.sqrt(v + eps)


def _dot(a, b):
    return jnp.dot(a, b, preferred_element_type=F32)


def _dot_nt(a, b):
    return jax.lax.dot_general(a, b, (((1,), (1,)), ((), ())), preferred_element_type=F32)


def _spread(items, n):
    return [items[(len(items) * i) // n:(len(items) * (i + 1)) // n] for i in range(n)]


def make(prio='01', fine=True, nochecks=True, wprio='01', gran=1, tail_split=(0.5,), compute=True, W2C=4):
    HG = 8
    NSLOT = 3

    def fn(A_x, A_k_cache, A_v_cache, A_wq, A_wo, B_x, B_w1, B_b1, B_w2, B_b2, c, w_mod):
        B, Sq, D = A_x.shape
        _, H, Sk, Dh = A_k_cache.shape
        Fh = B_w1.shape[1]
        W = min(4096, max(256, Sk // 4))
        R = HG * Dh
        NG = H // HG
        NSTEP = NG * B
        NT = R // 128
        scale = Dh ** -0.5

        def kernel(x_hbm, k_hbm, v_hbm, wq_hbm, wo_hbm, w1_hbm, b1_hbm, w2_hbm, b2_hbm, c_hbm, wmod_hbm,
                   out_ref,
                   x_v, c_v, b1_v, b2_v, wmod_v, wq_v, wo_v, w1_v, w2_v, kv_v, q_v, o_v,
                   sem_s, sem_w, sem_w2, sem_kv):
            def start_all(descs, pat):
                for i, cp in enumerate(descs):
                    cp.start(priority=int(pat[i % len(pat)]))

            def kv_descs(step, slot):
                g = step // B
                b = step % B
                out = []
                for r in range(Dh // 8):
                    for hp in range(HG // 2):
                        for i, src in enumerate((k_hbm, v_hbm)):
                            out.append(pltpu.make_async_copy(
                                src.at[b, pl.ds(g * HG + 2 * hp, 2), pl.ds(8 * r, 8), pl.ds(Sk - W, W)],
                                kv_v.at[slot, i, pl.ds(2 * hp, 2), pl.ds(8 * r, 8), :],
                                sem_kv.at[slot]))
                return out

            def w_descs(src, dst, sem, rows, cols, ns=8):
                _, n, m = src.shape
                nr = n // rows
                assert nr % ns == 0 and m % cols == 0
                out = []
                for r in range(nr // ns):
                    for cc in range(m // cols):
                        for s in range(ns):
                            r0 = (s * (nr // ns) + r) * rows
                            idx = (slice(None), pl.ds(r0, rows), pl.ds(cc * cols, cols))
                            out.append(pltpu.make_async_copy(src.at[idx], dst.at[idx], sem))
                return out

            def wait_all(buf, sem):
                pltpu.make_async_copy(buf, buf, sem).wait()

            small = [pltpu.make_async_copy(s, d, sem_s.at[i]) for i, (s, d) in enumerate(
                ((c_hbm, c_v), (x_hbm, x_v), (b1_hbm, b1_v), (b2_hbm, b2_v)))]
            d_mod = w_descs(wmod_hbm, wmod_v, sem_w.at[0], 8, 768)
            d_wq = w_descs(wq_hbm, wq_v, sem_w.at[1], 8, 1024)
            d_wo = w_descs(wo_hbm, wo_v, sem_w.at[2], 8, D)
            d_w1 = w_descs(w1_hbm, w1_v, sem_w.at[3], 8, 768)
            d_w2 = [w_descs(w2_hbm.at[i], w2_v.at[i], sem_w2.at[i], 8, D, ns=4) for i in range(W2C)]

            for cp in small:
                cp.start()
            start_all(d_mod, wprio)
            start_all(d_wq[:len(d_wq) // 2], wprio)
            for cp in small:
                cp.wait()
            cc = c_v[...].astype(F32)
            sc = (cc * jax.nn.sigmoid(cc)).astype(BF16)
            x = x_v[...].astype(F32)
            xn = _layernorm(x)
            wait_all(wmod_v, sem_w.at[0])
            mod = _dot(sc, wmod_v[...].reshape(D, 6 * D))
            sa, ca, ga, sb, cb, gb = (mod[:, i * D:(i + 1) * D] for i in range(6))
            h = (xn * (1.0 + ca) + sa).astype(BF16)
            start_all(d_wq[len(d_wq) // 2:], wprio)
            start_all(kv_descs(0, 0), prio)
            wait_all(wq_v, sem_w.at[1])
            d1 = _spread(kv_descs(1, 1), NG)
            for g in range(NG):
                q_v[g] = _dot(h, wq_v[:, :, g * R:(g + 1) * R].reshape(D, R))
                start_all(d1[g], prio)

            def rows_of(slot, i, t):
                lo, hi = 128 * t, 128 * (t + 1)
                parts = []
                while lo < hi:
                    hh = lo // Dh
                    n = min(hi, (hh + 1) * Dh) - lo
                    parts.append(kv_v[slot, i, hh, pl.ds(lo - hh * Dh, n), :])
                    lo += n
                return parts[0] if len(parts) == 1 else jnp.concatenate(parts, axis=0)

            def attn_step(step, slot, descs, pat):
                g = step // B
                b = step % B
                groups = _spread(descs, 2 * NT // gran)
                row = jax.lax.broadcasted_iota(jnp.int32, (HG, R), 0)
                col = jax.lax.broadcasted_iota(jnp.int32, (HG, R), 1)
                diag = (col >= row * Dh) & (col < (row + 1) * Dh)
                qb = jnp.broadcast_to(q_v[g, pl.ds(b, 1), :], (HG, R))
                qd = jnp.where(diag, qb, 0.0).astype(BF16)
                wait_all(kv_v.at[slot], sem_kv.at[slot])
                if not compute:
                    start_all(descs, pat)
                    o_v[g, pl.ds(b, 1), :] = q_v[g, pl.ds(b, 1), :]
                    return
                if fine:
                    s = None
                    for t in range(NT):
                        part = _dot(qd[:, 128 * t:128 * (t + 1)], rows_of(slot, 0, t))
                        s = part if s is None else s + part
                        if t % gran == gran - 1:
                            start_all(groups[t // gran], pat)
                else:
                    s = _dot(qd, kv_v[slot, 0].reshape(R, W))
                    start_all(descs[:len(descs) // 2], pat)
                s = s * scale
                m = jnp.max(s, axis=-1, keepdims=True)
                e = jnp.exp(s - m)
                l = jnp.sum(e, axis=-1, keepdims=True)
                eb = e.astype(BF16)
                if fine:
                    parts = []
                    for t in range(NT):
                        parts.append(_dot_nt(eb, rows_of(slot, 1, t)))
                        if t % gran == gran - 1:
                            start_all(groups[(NT + t) // gran], pat)
                    o = jnp.concatenate(parts, axis=1)
                else:
                    o = _dot_nt(eb, kv_v[slot, 1].reshape(R, W))
                    start_all(descs[len(descs) // 2:], pat)
                o = jnp.where(diag, o / l, 0.0)
                o_v[g, pl.ds(b, 1), :] = jnp.sum(o, axis=0, keepdims=True)

            def body(step, carry):
                attn_step(step, step % NSLOT, kv_descs(step + 2, (step + 2) % NSLOT), prio)
                return carry

            jax.lax.fori_loop(0, NSTEP - 2, body, None)
            tail = d_wo + d_w1
            n0 = int(len(tail) * tail_split[0])
            attn_step(NSTEP - 2, (NSTEP - 2) % NSLOT, tail[:n0], wprio)
            attn_step(NSTEP - 1, (NSTEP - 1) % NSLOT, tail[n0:], wprio)

            wait_all(wo_v, sem_w.at[2])
            attn = None
            d2 = _spread([cp for ch in d_w2 for cp in ch], 2)
            for g in range(NG):
                half, off = divmod(g * R, H * Dh // 2)
                part = _dot(o_v[g].astype(BF16), wo_v[half, pl.ds(off, R), :])
                attn = part if attn is None else attn + part
                if g < 2:
                    start_all(d2[g], wprio)
            x1 = x + ga * attn
            h2 = _layernorm(x1) * (1.0 + cb) + sb
            y = _layernorm(h2).astype(BF16)
            wait_all(w1_v, sem_w.at[3])
            u = _dot(y, w1_v[...].reshape(D, Fh)) + b1_v[...].astype(F32)[None, :]
            u = jax.nn.gelu(u, approximate=True).astype(BF16)
            mlp = jnp.broadcast_to(b2_v[...].astype(F32)[None, :], (B, D))
            ch = Fh // W2C
            for i in range(W2C):
                wait_all(w2_v.at[i], sem_w2.at[i])
                mlp = mlp + _dot(u[:, i * ch:(i + 1) * ch], w2_v[i].reshape(ch, D))
            out_ref[...] = (x1 + gb * mlp).astype(out_ref.dtype)

        kt = jnp.swapaxes(A_k_cache, 2, 3)
        vt = jnp.swapaxes(A_v_cache, 2, 3)
        halves = lambda w: w.reshape(2, w.shape[0] // 2, w.shape[1])
        w2r = B_w2.reshape(W2C, 2, Fh // W2C // 2, D)
        out = pl.pallas_call(
            kernel,
            out_shape=jax.ShapeDtypeStruct((B, D), A_x.dtype),
            in_specs=[pl.BlockSpec(memory_space=pl.ANY)] * 11,
            out_specs=pl.BlockSpec(memory_space=pltpu.VMEM),
            scratch_shapes=[
                pltpu.VMEM((B, D), BF16), pltpu.VMEM((B, D), BF16),
                pltpu.VMEM((Fh,), BF16), pltpu.VMEM((D,), BF16),
                pltpu.VMEM((2, D // 2, 6 * D), BF16), pltpu.VMEM((2, D // 2, H * Dh), BF16),
                pltpu.VMEM((2, H * Dh // 2, D), BF16),
                pltpu.VMEM((2, D // 2, Fh), BF16), pltpu.VMEM(w2r.shape, BF16),
                pltpu.VMEM((NSLOT, 2, HG, Dh, W), BF16),
                pltpu.VMEM((NG, B, R), F32), pltpu.VMEM((NG, B, R), F32),
                pltpu.SemaphoreType.DMA((4,)), pltpu.SemaphoreType.DMA((4,)), pltpu.SemaphoreType.DMA((W2C,)),
                pltpu.SemaphoreType.DMA((NSLOT,)),
            ],
            compiler_params=pltpu.CompilerParams(vmem_limit_bytes=100 * 1024 * 1024,
                                                 disable_bounds_checks=nochecks, disable_semaphore_checks=nochecks),
        )(A_x.reshape(B, D), kt, vt, halves(A_wq), halves(A_wo), halves(B_w1), B_b1, w2r, B_b2, c, halves(w_mod))
        return out.reshape(B, Sq, D)
    return fn


_impl = make()


@jax.jit
def pallas_adaLN_cond__sliding_block_cached__mixer_channel_mlp__decode_kernel(
    A_x, A_k_cache, A_v_cache, A_wq, A_wo, B_x, B_w1, B_b1, B_w2, B_b2, c, w_mod
):
    return _impl(A_x, A_k_cache, A_v_cache, A_wq, A_wo, B_x, B_w1, B_b1, B_w2, B_b2, c, w_mod)
```

```python
import functools
import jax
import jax.numpy as jnp
from jax.experimental import pallas as pl
from jax.experimental.pallas import tpu as pltpu

F32 = jnp.float32
BF16 = jnp.bfloat16


def _layernorm(x, eps=1e-5):
    m = jnp.mean(x, axis=-1, keepdims=True)
    d = x - m
    v = jnp.mean(d * d, axis=-1, keepdims=True)
    return d / jnp.sqrt(v + eps)


def _dot(a, b):
    return jnp.dot(a, b, preferred_element_type=F32)


def _dot_nt(a, b):
    return jax.lax.dot_general(a, b, (((1,), (1,)), ((), ())), preferred_element_type=F32)


def make(nochecks=True, W2CH=(384, 384, 384, 384), rsplit=3, dma_only=False, wo_ns=16, w2_ns=4, mod_cfg=(1920, 20, 1),
         wq_cfg=(1024, 8, 2), w1_cfg=(1536, 8, 1), rot=0, krot=0, w2pts=(0, 1, 2, 3), wo_rows=24, w2_rows=24):
    HG = 8
    NSLOT = 3

    def fn(A_x, A_k_cache, A_v_cache, A_wq, A_wo, B_x, B_w1, B_b1, B_w2, B_b2, c, w_mod):
        B, Sq, D = A_x.shape
        _, H, Sk, Dh = A_k_cache.shape
        Fh = B_w1.shape[1]
        W = min(4096, max(256, Sk // 4))
        R = HG * Dh
        NG = H // HG
        NSTEP = NG * B
        scale = Dh ** -0.5
        w2_off = [sum(W2CH[:i]) for i in range(len(W2CH))]

        def kernel(x_hbm, k_hbm, v_hbm, wq_hbm, wo_hbm, w1_hbm, b1_hbm, w2_hbm, b2_hbm, c_hbm, wmod_hbm,
                   out_ref,
                   x_v, c_v, b1_v, b2_v, wmod_v, wq_v, wo_v, w1_v, w2_v, kv_v, q_v, o_v,
                   sem_s, sem_w, sem_w2, sem_kv):
            def start_all(descs):
                for i, cp in enumerate(descs):
                    cp.start(priority=i % 2)

            def kv_descs(step):
                slot = step % NSLOT
                g = step // B
                b = step % B
                out = []
                nr = Dh // 8
                for r0 in range(nr // rsplit):
                    for s in range(rsplit):
                        for hp in range(HG // 2):
                            for i, src in enumerate((k_hbm, v_hbm)):
                                r = (r0 + s * (nr // rsplit) + rot * hp + krot * i) % nr
                                out.append(pltpu.make_async_copy(
                                    src.at[b, pl.ds(g * HG + 2 * hp, 2), pl.ds(8 * r, 8), pl.ds(Sk - W, W)],
                                    kv_v.at[slot, i, pl.ds(2 * hp, 2), pl.ds(8 * r, 8), :],
                                    sem_kv.at[slot]))
                return out

            def wide_start(src, dst, sem, cols, ns, lo=0.0, hi=1.0):
                _, n, m = src.shape
                nr, nc = n // 8, m // cols
                assert nr % ns == 0 and m % cols == 0
                trips = nr // ns * nc

                @pl.loop(int(lo * trips), int(hi * trips))
                def _(i):
                    r, cc = i // nc, i % nc
                    for s in range(ns):
                        idx = (slice(None), pl.ds(pl.multiple_of((s * (nr // ns) + r) * 8, 8), 8),
                               pl.ds(pl.multiple_of(cc * cols, 128), cols))
                        pltpu.make_async_copy(src.at[idx], dst.at[idx], sem).start(priority=s % 2)

            def tall_start(src, dst, sem, off, n, rows, ns, lo=0.0, hi=1.0):
                nr = n // rows
                assert n % rows == 0 and nr % ns == 0, (n, rows, ns)
                trips = nr // ns

                @pl.loop(int(lo * trips), int(hi * trips))
                def _(r):
                    for s in range(ns):
                        idx = pl.ds(pl.multiple_of(off + (s * (nr // ns) + r) * rows, 8), rows)
                        pltpu.make_async_copy(src.at[idx], dst.at[idx], sem).start(priority=s % 2)

            def wait_all(buf, sem):
                pltpu.make_async_copy(buf, buf, sem).wait()

            small = [pltpu.make_async_copy(s, d, sem_s.at[i]) for i, (s, d) in enumerate(
                ((c_hbm, c_v), (x_hbm, x_v), (b1_hbm, b1_v), (b2_hbm, b2_v)))]

            start_all(small)
            wide_start(wmod_hbm, wmod_v, sem_w.at[0], *mod_cfg[:2])
            wide_start(wq_hbm, wq_v, sem_w.at[1], *wq_cfg[:2], hi=0.5)
            for cp in small:
                cp.wait()
            cc = c_v[...].astype(F32)
            sc = (cc * jax.nn.sigmoid(cc)).astype(BF16)
            x = x_v[...].astype(F32)
            xn = _layernorm(x)
            wait_all(wmod_v, sem_w.at[0])
            if not dma_only:
                mod = _dot(sc, wmod_v[...].reshape(D, 6 * D))
                sa, ca, ga, sb, cb, gb = (mod[:, i * D:(i + 1) * D] for i in range(6))
                h = (xn * (1.0 + ca) + sa).astype(BF16)
            wide_start(wq_hbm, wq_v, sem_w.at[1], *wq_cfg[:2], lo=0.5)

            @pl.loop(0, NSLOT - 1)
            def _(step):
                descs = kv_descs(step)
                half = len(descs) // 2
                start_all(descs[:half])

                @pl.when(step == 0)
                def _():
                    wait_all(wq_v, sem_w.at[1])

                if not dma_only:
                    for j in range(NG // (NSLOT - 1)):
                        g = step * (NG // (NSLOT - 1)) + j
                        q_v[g] = _dot(h, wq_v[:, :, pl.ds(pl.multiple_of(g * R, 128), R)].reshape(D, R))
                start_all(descs[half:])

            def attn_step(step, first, second):
                slot = step % NSLOT
                g = step // B
                b = step % B
                if dma_only:
                    wait_all(kv_v.at[slot], sem_kv.at[slot])
                    first()
                    second()
                    return
                row = jax.lax.broadcasted_iota(jnp.int32, (HG, R), 0)
                col = jax.lax.broadcasted_iota(jnp.int32, (HG, R), 1)
                diag = (col >= row * Dh) & (col < (row + 1) * Dh)
                qb = jnp.broadcast_to(q_v[g, pl.ds(b, 1), :], (HG, R))
                qd = jnp.where(diag, qb, 0.0).astype(BF16)
                wait_all(kv_v.at[slot], sem_kv.at[slot])
                s = _dot(qd, kv_v[slot, 0].reshape(R, W)) * scale
                first()
                m = jnp.max(s, axis=-1, keepdims=True)
                e = jnp.exp(s - m)
                l = jnp.sum(e, axis=-1, keepdims=True)
                o = _dot_nt(e.astype(BF16), kv_v[slot, 1].reshape(R, W))
                second()
                o = jnp.where(diag, o / l, 0.0)
                o_v[g, pl.ds(b, 1), :] = jnp.sum(o, axis=0, keepdims=True)

            @pl.loop(0, NSTEP - 2)
            def _(step):
                descs = kv_descs(step + 2)
                half = len(descs) // 2
                attn_step(step, lambda: start_all(descs[:half]), lambda: start_all(descs[half:]))

            wo_start = functools.partial(tall_start, wo_hbm, wo_v, sem_w.at[2], 0, H * Dh, wo_rows, wo_ns)
            attn_step(NSTEP - 2, lambda: wo_start(0.0, 0.375), lambda: wo_start(0.375, 0.75))
            attn_step(NSTEP - 1, lambda: wo_start(0.75, 1.0),
                      lambda: wide_start(w1_hbm, w1_v, sem_w.at[3], *w1_cfg[:2]))

            wait_all(wo_v, sem_w.at[2])
            attn = None
            todo = list(enumerate(zip(w2_off, W2CH)))
            for g in range(NG):
                if not dma_only:
                    part = _dot(o_v[g].astype(BF16), wo_v[pl.ds(g * R, R), :])
                    attn = part if attn is None else attn + part
                for i, (o, n) in todo:
                    if w2pts[i] == g:
                        rows, ns = (w2_rows, w2_ns) if n % (w2_rows * w2_ns) == 0 else (16, 8)
                        tall_start(w2_hbm, w2_v, sem_w2.at[i], o, n, rows, ns)
            if dma_only:
                wait_all(w1_v, sem_w.at[3])
                for i, (o, n) in todo:
                    wait_all(w2_v.at[pl.ds(o, n)], sem_w2.at[i])
                out_ref[...] = x_v[...]
                return
            x1 = x + ga * attn
            h2 = _layernorm(x1) * (1.0 + cb) + sb
            y = _layernorm(h2).astype(BF16)
            wait_all(w1_v, sem_w.at[3])
            u = _dot(y, w1_v[...].reshape(D, Fh)) + b1_v[...].astype(F32)[None, :]
            u = jax.nn.gelu(u, approximate=True).astype(BF16)
            mlp = jnp.broadcast_to(b2_v[...].astype(F32)[None, :], (B, D))
            for i, (o, n) in todo:
                wait_all(w2_v.at[pl.ds(o, n)], sem_w2.at[i])
                mlp = mlp + _dot(u[:, o:o + n], w2_v[pl.ds(o, n), :])
            out_ref[...] = (x1 + gb * mlp).astype(out_ref.dtype)

        kt = jnp.swapaxes(A_k_cache, 2, 3)
        vt = jnp.swapaxes(A_v_cache, 2, 3)
        split = lambda w, p: w.reshape(p, w.shape[0] // p, w.shape[1])
        wmod3, wq3, w13 = split(w_mod, mod_cfg[2]), split(A_wq, wq_cfg[2]), split(B_w1, w1_cfg[2])
        out = pl.pallas_call(
            kernel,
            out_shape=jax.ShapeDtypeStruct((B, D), A_x.dtype),
            in_specs=[pl.BlockSpec(memory_space=pl.ANY)] * 11,
            out_specs=pl.BlockSpec(memory_space=pltpu.VMEM),
            scratch_shapes=[
                pltpu.VMEM((B, D), BF16), pltpu.VMEM((B, D), BF16),
                pltpu.VMEM((Fh,), BF16), pltpu.VMEM((D,), BF16),
                pltpu.VMEM(wmod3.shape, BF16), pltpu.VMEM(wq3.shape, BF16),
                pltpu.VMEM((H * Dh, D), BF16),
                pltpu.VMEM(w13.shape, BF16), pltpu.VMEM((Fh, D), BF16),
                pltpu.VMEM((NSLOT, 2, HG, Dh, W), BF16),
                pltpu.VMEM((NG, B, R), F32), pltpu.VMEM((NG, B, R), F32),
                pltpu.SemaphoreType.DMA((4,)), pltpu.SemaphoreType.DMA((4,)), pltpu.SemaphoreType.DMA((len(W2CH),)),
                pltpu.SemaphoreType.DMA((NSLOT,)),
            ],
            compiler_params=pltpu.CompilerParams(vmem_limit_bytes=100 * 1024 * 1024,
                                                 disable_bounds_checks=nochecks, disable_semaphore_checks=nochecks),
        )(A_x.reshape(B, D), kt, vt, wq3, A_wo, w13, B_b1, B_w2, B_b2, c, wmod3)
        return out.reshape(B, Sq, D)
    return fn


_impl = make(W2CH=(768,384,384), w2pts=(1,2,3))


@jax.jit
def pallas_adaLN_cond__sliding_block_cached__mixer_channel_mlp__decode_kernel(
    A_x, A_k_cache, A_v_cache, A_wq, A_wo, B_x, B_w1, B_b1, B_w2, B_b2, c, w_mod
):
    return _impl(A_x, A_k_cache, A_v_cache, A_wq, A_wo, B_x, B_w1, B_b1, B_w2, B_b2, c, w_mod)
```

```python
import jax
import jax.numpy as jnp
from jax.experimental import pallas as pl
from jax.experimental.pallas import tpu as pltpu

F32 = jnp.float32
BF16 = jnp.bfloat16

HEADS_PER_STEP = 8
KV_SLOTS = 3
TILE_ROWS = 8
W2_CHUNKS = (768, 384, 384)


def _layernorm(x, eps=1e-5):
    m = jnp.mean(x, axis=-1, keepdims=True)
    d = x - m
    v = jnp.mean(d * d, axis=-1, keepdims=True)
    return d / jnp.sqrt(v + eps)


def _dot(a, b):
    return jnp.dot(a, b, preferred_element_type=F32)


def _dot_nt(a, b):
    return jax.lax.dot_general(a, b, (((1,), (1,)), ((), ())), preferred_element_type=F32)


def _start(copies):
    for i, cp in enumerate(copies):
        cp.start(priority=i % 2)


def _wait_filled(buf, sem):
    pltpu.make_async_copy(buf, buf, sem).wait()


def _start_wide(arrays, n_col, streams):
    per_stream = arrays[0][0].shape[1] // TILE_ROWS // streams

    @pl.loop(0, per_stream * n_col)
    def _(i):
        r, c = i // n_col, i % n_col
        copies = []
        for s in range(streams):
            rows = pl.ds(pl.multiple_of((s * per_stream + r) * TILE_ROWS, TILE_ROWS), TILE_ROWS)
            for src, dst, sem in arrays:
                width = src.shape[2] // n_col
                idx = (slice(None), rows, pl.ds(pl.multiple_of(c * width, 128), width))
                copies.append(pltpu.make_async_copy(src.at[idx], dst.at[idx], sem))
        _start(copies)


def _start_tall(src, dst, sem, offset, n, streams, lo=0.0, hi=1.0):
    height = 3 * TILE_ROWS
    per_stream = n // height // streams
    assert per_stream * height * streams == n

    @pl.loop(int(lo * per_stream), int(hi * per_stream))
    def _(r):
        copies = []
        for s in range(streams):
            rows = pl.ds(pl.multiple_of(offset + (s * per_stream + r) * height, TILE_ROWS), height)
            copies.append(pltpu.make_async_copy(src.at[rows], dst.at[rows], sem))
        _start(copies)


def _kernel(x_hbm, k_hbm, v_hbm, wq_hbm, wo_hbm, w1_hbm, b1_hbm, w2_hbm, b2_hbm, c_hbm, wmod_hbm,
            out_ref,
            x_v, c_v, b1_v, b2_v, wmod_v, wq_v, wo_v, w1_v, w2_v, kv_v, q_v, o_v,
            sem_small, sem_w, sem_w2, sem_kv):
    B, D = x_v.shape
    _, H, Dh, Sk = k_hbm.shape
    W = kv_v.shape[-1]
    F = w2_v.shape[0]
    HG = HEADS_PER_STEP
    R = HG * Dh
    n_groups = H // HG
    n_steps = n_groups * B

    def kv_copies(step):
        slot, g, b = step % KV_SLOTS, step // B, step % B
        n = Dh // TILE_ROWS
        copies = []
        for r0 in range(n // 3):
            for third in range(3):
                for h in range(0, HG, 2):
                    for i, src in enumerate((k_hbm, v_hbm)):
                        rows = pl.ds((r0 + third * (n // 3) + 2 * i) % n * TILE_ROWS, TILE_ROWS)
                        copies.append(pltpu.make_async_copy(
                            src.at[b, pl.ds(g * HG + h, 2), rows, pl.ds(Sk - W, W)],
                            kv_v.at[slot, i, pl.ds(h, 2), rows, :],
                            sem_kv.at[slot]))
        return copies[:len(copies) // 2], copies[len(copies) // 2:]

    small = [pltpu.make_async_copy(src, dst, sem_small.at[i]) for i, (src, dst) in enumerate(
        ((c_hbm, c_v), (x_hbm, x_v), (b1_hbm, b1_v), (b2_hbm, b2_v)))]
    _start(small)
    _start_wide(((wmod_hbm, wmod_v, sem_w.at[0]), (wq_hbm, wq_v, sem_w.at[1])), n_col=6, streams=4)
    kv0, kv1 = kv_copies(0), kv_copies(1)
    _start(kv0[0])
    for cp in small:
        cp.wait()
    c = c_v[...].astype(F32)
    silu_c = (c * jax.nn.sigmoid(c)).astype(BF16)
    x = x_v[...].astype(F32)
    _wait_filled(wmod_v, sem_w.at[0])
    mod = _dot(silu_c, wmod_v[...].reshape(D, 6 * D))
    sa, ca, ga, sb, cb, gb = (mod[:, i * D:(i + 1) * D] for i in range(6))
    h = (_layernorm(x) * (1.0 + ca) + sa).astype(BF16)
    _start(kv0[1])
    _wait_filled(wq_v, sem_w.at[1])
    for g in range(n_groups):
        q_v[g] = _dot(h, wq_v[:, :, g * R:(g + 1) * R].reshape(D, R))
        if g % 2 == 1:
            _start(kv1[g // 2])

    def attend(step, fetch_a, fetch_b):
        slot, g, b = step % KV_SLOTS, step // B, step % B
        row = jax.lax.broadcasted_iota(jnp.int32, (HG, R), 0)
        col = jax.lax.broadcasted_iota(jnp.int32, (HG, R), 1)
        diag = (col >= row * Dh) & (col < (row + 1) * Dh)
        q = jnp.broadcast_to(q_v[g, pl.ds(b, 1), :], (HG, R))
        q = jnp.where(diag, q, 0.0).astype(BF16)
        _wait_filled(kv_v.at[slot], sem_kv.at[slot])
        s = _dot(q, kv_v[slot, 0].reshape(R, W)) * Dh ** -0.5
        fetch_a()
        p = jnp.exp(s - jnp.max(s, axis=-1, keepdims=True))
        denom = jnp.sum(p, axis=-1, keepdims=True)
        o = _dot_nt(p.astype(BF16), kv_v[slot, 1].reshape(R, W))
        fetch_b()
        o_v[g, pl.ds(b, 1), :] = jnp.sum(jnp.where(diag, o / denom, 0.0), axis=0, keepdims=True)

    @pl.loop(0, n_steps - 2)
    def _(step):
        ahead = kv_copies(step + 2)
        attend(step, lambda: _start(ahead[0]), lambda: _start(ahead[1]))

    def fetch_wo(lo, hi):
        return lambda: _start_tall(wo_hbm, wo_v, sem_w.at[2], 0, H * Dh, 8, lo, hi)

    attend(n_steps - 2, fetch_wo(0.0, 0.375), fetch_wo(0.375, 0.75))
    attend(n_steps - 1, fetch_wo(0.75, 1.0),
           lambda: _start_wide(((w1_hbm, w1_v, sem_w.at[3]),), n_col=3, streams=2))

    chunks = [(sum(W2_CHUNKS[:i]), n) for i, n in enumerate(W2_CHUNKS)]
    _wait_filled(wo_v, sem_w.at[2])
    attn = jnp.zeros((B, D), F32)
    for g in range(n_groups):
        attn += _dot(o_v[g].astype(BF16), wo_v[g * R:(g + 1) * R, :])
        if g > 0:
            _start_tall(w2_hbm, w2_v, sem_w2.at[g - 1], *chunks[g - 1], 4)
    x = x + ga * attn
    y = _layernorm(_layernorm(x) * (1.0 + cb) + sb).astype(BF16)
    _wait_filled(w1_v, sem_w.at[3])
    u = _dot(y, w1_v[...].reshape(D, F)) + b1_v[...].astype(F32)[None, :]
    u = jax.nn.gelu(u, approximate=True).astype(BF16)
    mlp = jnp.broadcast_to(b2_v[...].astype(F32)[None, :], (B, D))
    for i, (lo, n) in enumerate(chunks):
        _wait_filled(w2_v.at[pl.ds(lo, n)], sem_w2.at[i])
        mlp += _dot(u[:, lo:lo + n], w2_v[lo:lo + n, :])
    out_ref[...] = (x + gb * mlp).astype(out_ref.dtype)


@jax.jit
def pallas_adaLN_cond__sliding_block_cached__mixer_channel_mlp__decode_kernel(
    A_x: jax.Array,
    A_k_cache: jax.Array,
    A_v_cache: jax.Array,
    A_wq: jax.Array,
    A_wo: jax.Array,
    B_x: jax.Array,
    B_w1: jax.Array,
    B_b1: jax.Array,
    B_w2: jax.Array,
    B_b2: jax.Array,
    c: jax.Array,
    w_mod: jax.Array,
):
    del B_x
    B, Sq, D = A_x.shape
    _, H, Sk, Dh = A_k_cache.shape
    F = B_w1.shape[1]
    W = min(4096, max(256, Sk // 4))
    n_groups, R = H // HEADS_PER_STEP, HEADS_PER_STEP * Dh
    assert Sq == 1 and n_groups == len(W2_CHUNKS) + 1 and F == sum(W2_CHUNKS)

    def split_rows(w, parts):
        return w.reshape(parts, w.shape[0] // parts, w.shape[1])

    wmod, wq, w1 = split_rows(w_mod, 2), split_rows(A_wq, 2), split_rows(B_w1, 4)
    out = pl.pallas_call(
        _kernel,
        out_shape=jax.ShapeDtypeStruct((B, D), A_x.dtype),
        in_specs=[pl.BlockSpec(memory_space=pl.ANY)] * 11,
        out_specs=pl.BlockSpec(memory_space=pltpu.VMEM),
        scratch_shapes=[
            pltpu.VMEM((B, D), BF16),
            pltpu.VMEM((B, D), BF16),
            pltpu.VMEM((F,), BF16),
            pltpu.VMEM((D,), BF16),
            pltpu.VMEM(wmod.shape, BF16),
            pltpu.VMEM(wq.shape, BF16),
            pltpu.VMEM(A_wo.shape, BF16),
            pltpu.VMEM(w1.shape, BF16),
            pltpu.VMEM(B_w2.shape, BF16),
            pltpu.VMEM((KV_SLOTS, 2, HEADS_PER_STEP, Dh, W), BF16),
            pltpu.VMEM((n_groups, B, R), F32),
            pltpu.VMEM((n_groups, B, R), F32),
            pltpu.SemaphoreType.DMA((4,)),
            pltpu.SemaphoreType.DMA((4,)),
            pltpu.SemaphoreType.DMA((len(W2_CHUNKS),)),
            pltpu.SemaphoreType.DMA((KV_SLOTS,)),
        ],
        compiler_params=pltpu.CompilerParams(
            vmem_limit_bytes=64 * 1024 * 1024,
            disable_semaphore_checks=True,
        ),
    )(A_x.reshape(B, D), jnp.swapaxes(A_k_cache, 2, 3), jnp.swapaxes(A_v_cache, 2, 3),
      wq, A_wo, w1, B_b1, B_w2, B_b2, c, wmod)
    return out.reshape(B, Sq, D)
```
